```python
import os as _os
_os.environ.setdefault("JAX_PLATFORMS", "cpu")
import jax
import jax.numpy as jnp

def _softmax(x, axis=-1):
    return jax.nn.softmax(x, axis=axis)
def _gelu(x):
    return jax.nn.gelu(x, approximate=True)
def _silu(x):
    return jax.nn.silu(x)
def _sigmoid(x):
    return jax.nn.sigmoid(x)
def _layernorm(x, axis=-1, eps=1e-5):
    m = jnp.mean(x, axis=axis, keepdims=True)
    v = jnp.var(x, axis=axis, keepdims=True)
    return (x - m) / jnp.sqrt(v + eps)
def _scatter_add(tgt, idx, src, axis=0):
    return tgt.at[idx].add(src)
def _segment_sum(src, seg, n):
    return jax.ops.segment_sum(src, seg, n)
class _Rng:
    def __init__(self, key):
        self._k = key
    def _next(self):
        self._k, sub = jax.random.split(self._k)
        return sub
    def normal(self, shape):
        return jax.random.normal(self._next(), shape, dtype=jnp.bfloat16)
    def randint(self, lo, hi, shape):
        return jax.random.randint(self._next(), shape, lo, hi, dtype=jnp.int32)
    def uniform(self, shape, lo=0.0, hi=1.0):
        return jax.random.uniform(self._next(), shape, jnp.bfloat16, lo, hi)
    def permutation(self, n):
        return jax.random.permutation(self._next(), n)


kernel_name = 'parallel_sum__ssm_conv_s4__mixer_channel_mlp__prompt'

def setup_inputs():
    _rng = _Rng(jax.random.key(int.from_bytes(__import__("os").urandom(4), "little")))
    _w = (lambda a: (lambda t: t.astype(jnp.bfloat16) if jnp.issubdtype(t.dtype, jnp.floating) else t)(jnp.asarray(a)))
    def _A_setup():
        B, L, D, N = 1, 2048, 512, 128
        A_re = -jnp.exp((lambda *s: _rng.normal(s) * 0.1)(D, N))
        A_im = jnp.pi * (lambda *s: _rng.normal(s) * 0.1)(D, N)
        B_re = (lambda *s: _rng.normal(s) * 0.1)(D, N)
        B_im = (lambda *s: _rng.normal(s) * 0.1)(D, N)
        C_re = (lambda *s: _rng.normal(s) * 0.1)(D, N)
        C_im = (lambda *s: _rng.normal(s) * 0.1)(D, N)
        log_dt = (lambda *s: _rng.normal(s) * 0.1)(D) * 0.5 - 4.0
        Dskip = (lambda *s: _rng.normal(s) * 0.05)(D)
        return {
            "u": _w((lambda *s: _rng.normal(s) * 0.05)(B, L, D)),
            "A_re": _w(A_re),
            "A_im": _w(A_im),
            "B_re": _w(B_re),
            "B_im": _w(B_im),
            "C_re": _w(C_re),
            "C_im": _w(C_im),
            "log_dt": _w(log_dt),
            "Dskip": _w(Dskip),
        }
    _A_in = _A_setup()

    def _B_setup():
        B, S, D, F = 1, 2048, 512, 1792
        return {
            "x": _w((lambda *s: _rng.normal(s) * 0.05)(B, S, D)),
            "w1": _w((lambda *s: _rng.normal(s) * 0.2)(D, F) * (D ** -0.5)),
            "b1": _w((lambda *s: _rng.normal(s) * 0.2)(F)),
            "w2": _w((lambda *s: _rng.normal(s) * 0.2)(F, D) * (F ** -0.5)),
            "b2": _w((lambda *s: _rng.normal(s) * 0.05)(D)),
        }
    _B_in = _B_setup()

    return {
        "A_u": _A_in["u"],
        "A_A_re": _A_in["A_re"],
        "A_A_im": _A_in["A_im"],
        "A_B_re": _A_in["B_re"],
        "A_B_im": _A_in["B_im"],
        "A_C_re": _A_in["C_re"],
        "A_C_im": _A_in["C_im"],
        "A_log_dt": _A_in["log_dt"],
        "A_Dskip": _A_in["Dskip"],
        "B_x": _B_in["x"],
        "B_w1": _B_in["w1"],
        "B_b1": _B_in["b1"],
        "B_w2": _B_in["w2"],
        "B_b2": _B_in["b2"],
    }

def reference(A_u, A_A_re, A_A_im, A_B_re, A_B_im, A_C_re, A_C_im, A_log_dt, A_Dskip, B_x, B_w1, B_b1, B_w2, B_b2):
    def _A_ref(u, A_re, A_im, B_re, B_im, C_re, C_im, log_dt, Dskip):
        Bsz, L, D = u.shape
        dt = jnp.exp(log_dt)[:, None]
        A = A_re + 1j * A_im
        Bc = B_re + 1j * B_im
        Cc = C_re + 1j * C_im
        logdA = dt * A
        dB = dt * Bc
        l = (lambda x, dt: x.astype(dt))(jnp.arange(L), A_re.dtype)
        P = jnp.exp(logdA[:, :, None] * l[None, None, :])
        K = jnp.einsum("dn,dnl,dn->dl", Cc, P, dB).real
        L2 = 2 * L
        Kp = jnp.pad(K, ((0, 0), (0, L)))
        up = (lambda x, *d: x.transpose(*d))(u, 0, 2, 1)
        up = jnp.pad(up, ((0, 0), (0, 0), (0, L)))
        Kf = (lambda x, axes=(-2,-1): jnp.fft.rfft2(x.astype(jnp.float32), axes=axes))(Kp[:, None, :], axes=(-2, -1))
        Uf = (lambda x, axes=(-2,-1): jnp.fft.rfft2(x.astype(jnp.float32), axes=axes))(up[:, :, None, :], axes=(-2, -1))
        Yf = Uf * Kf[None, :, :, :]
        y = (lambda x, s, axes=(-2,-1): jnp.fft.irfft2(x, s=s, axes=axes).astype(jnp.bfloat16))(Yf, (1, L2), axes=(-2, -1))[:, :, 0, :L]
        y = (lambda x, *d: x.transpose(*d))(y, 0, 2, 1) + u * Dskip[None, None, :]
        return y

    def _B_ref(x, w1, b1, w2, b2):
        y = _layernorm(x, axis=-1)
        h = _gelu(jnp.einsum("bsd,df->bsf", y, w1) + b1)
        return jnp.einsum("bsf,fd->bsd", h, w2) + b2

    x = A_u
    xn = _layernorm(x, axis=-1)
    return x + _A_ref(xn, A_A_re, A_A_im, A_B_re, A_B_im, A_C_re, A_C_im, A_log_dt, A_Dskip) + _B_ref(xn, B_w1, B_b1, B_w2, B_b2)
```

```python
import numpy as np
import jax
import jax.numpy as jnp
from jax import lax
import jax.experimental.pallas as pl
import jax.experimental.pallas.tpu as pltpu

L, D, N, F = 2048, 512, 128, 1792
BLK = 256
NSTEP = L // BLK
CH = D // NSTEP
S = 4
f32, bf16 = jnp.float32, jnp.bfloat16

ROWS = [(r, i) for i in (0, 1) for r in range(8)] + [(r, i) for i in (2, 3) for r in (0, 2, 4, 6)] + \
       [(r, i) for i in range(4, 8) for r in (0, 4)] + [(0, i) for i in range(8, 17)]
NQ = len(ROWS)
NA = (NQ + 7) // 8


def _bf16_round_int(v):
    if v < 256:
        return v
    sh = v.bit_length() - 8
    q, rem = v >> sh, v & ((1 << sh) - 1)
    half = 1 << (sh - 1)
    if rem > half or (rem == half and (q & 1)):
        q += 1
    return q << sh


def _src_rows():
    pos = {}
    for q, (r, i) in enumerate(ROWS):
        a, p = divmod(q, 8)
        for j in range(16):
            pos[8 * (16 * i + j) + r] = a * 128 + 8 * j + p
    return [pos[_bf16_round_int(l)] for l in range(L)]


SRC = _src_rows()


def _dft_consts():
    n1 = np.arange(32); k1 = np.arange(33)
    F1 = np.zeros((66, 32))
    ang = 2 * np.pi * np.outer(k1, n1) / 64
    F1[0::2] = np.cos(ang); F1[1::2] = -np.sin(ang)
    n2 = np.arange(64); k2 = np.arange(64)
    G = np.zeros((33, 128, 128)); Gi = np.zeros((33, 128, 128))
    for a in range(33):
        th = 2 * np.pi * np.outer(a + 64 * k2, n2) / 4096
        G[a, :64, :64] = np.cos(th); G[a, :64, 64:] = np.sin(th)
        G[a, 64:, :64] = -np.sin(th); G[a, 64:, 64:] = np.cos(th)
        thi = th.T
        Gi[a, :64, :64] = np.cos(thi); Gi[a, :64, 64:] = -np.sin(thi)
        Gi[a, 64:, :64] = np.sin(thi); Gi[a, 64:, 64:] = np.cos(thi)
    Fi = np.zeros((32, 66))
    for a in range(33):
        w = 1.0 if a in (0, 32) else 2.0
        ph = 2 * np.pi * a * n1 / 64
        Fi[:, 2 * a] = w * np.cos(ph) / 4096; Fi[:, 2 * a + 1] = -w * np.sin(ph) / 4096
    F1S = np.zeros((66 * S, 32 * S)); FiS = np.zeros((32 * S, 384))
    for a in range(S):
        F1S[a::S, a::S] = F1
        FiS[a::S, a:66 * S:S] = Fi
    return F1S, G, Gi, FiS


def _ln(a):
    m = jnp.mean(a, axis=-1, keepdims=True)
    c = a - m
    v = jnp.mean(c * c, axis=-1, keepdims=True)
    return c * lax.rsqrt(v + 1e-5)


def _cm(a, b):
    return (a[0] * b[0] - a[1] * b[1], a[0] * b[1] + a[1] * b[0])


def _kernel(x_ref, ldt_ref, are_ref, aim_ref, bre_ref, bim_ref, cre_ref, cim_ref, dk_ref,
            w1_ref, b1_ref, w2_ref, b2_ref, f1_ref, g_ref, gi_ref, fi_ref,
            o_ref,
            UK, ACC, E_s, F_s, Kd, KdT, Y1, Q):
    i = pl.program_id(0)

    r0 = pl.multiple_of(i * BLK, BLK)
    x = x_ref[...].astype(f32)
    xn = _ln(x).astype(bf16).astype(f32)
    y = _ln(xn).astype(bf16)
    h = jnp.dot(y, w1_ref[...], preferred_element_type=f32) + b1_ref[...].astype(f32)
    h = jax.nn.gelu(h, approximate=True).astype(bf16)
    m = jnp.dot(h, w2_ref[...], preferred_element_type=f32) + b2_ref[...].astype(f32)
    acc = x + xn * dk_ref[...].astype(f32) + m
    for t in range(4):
        UK[t, pl.ds(r0, BLK), :] = xn[:, t * 128:(t + 1) * 128]
        ACC[t, pl.ds(r0, BLK), :] = acc[:, t * 128:(t + 1) * 128]

    c0 = pl.multiple_of(i * CH, CH)
    dt = jnp.exp(ldt_ref[pl.ds(c0, CH), :].astype(f32)).astype(bf16).astype(f32)
    ar = dt * are_ref[pl.ds(c0, CH), :].astype(f32)
    ai = dt * aim_ref[pl.ds(c0, CH), :].astype(f32)
    br = dt * bre_ref[pl.ds(c0, CH), :].astype(f32)
    bi = dt * bim_ref[pl.ds(c0, CH), :].astype(f32)
    c = _cm((cre_ref[pl.ds(c0, CH), :].astype(f32), cim_ref[pl.ds(c0, CH), :].astype(f32)), (br, bi))
    e = jnp.exp(ar)
    z = (e * jnp.cos(ai), e * jnp.sin(ai))
    z2 = _cm(z, z); z4 = _cm(z2, z2); w = _cm(z4, z4)
    one = jnp.ones_like(ar); zero = jnp.zeros_like(ar)
    Fj = (one, zero); F8 = None
    for j in range(16):
        F_s[j, :, 0:N] = Fj[0]; F_s[j, :, N:2 * N] = Fj[1]
        if j == 8:
            F8 = Fj
        if j < 15:
            Fj = _cm(Fj, w)
    w16 = _cm(F8, F8)
    cz = [c]
    for r in range(7):
        cz.append(_cm(cz[-1], z))
    Wi = (one, zero); q = 0
    for ii in range(17):
        for (r, i2) in ROWS:
            if i2 == ii:
                E = _cm(cz[r], Wi)
                E_s[q, :, 0:N] = E[0]; E_s[q, :, N:2 * N] = -E[1]
                q += 1
        if ii < 16:
            Wi = _cm(Wi, w16)
    lane = lax.broadcasted_iota(jnp.int32, (8, 128), 1)
    diag = (lane % 8) == lax.broadcasted_iota(jnp.int32, (8, 128), 0)
    for g in range(CH // 8):
        lhs = E_s[:, g * 8:(g + 1) * 8, :].reshape(NQ * 8, 2 * N).astype(bf16)
        rhs = F_s[:, g * 8:(g + 1) * 8, :].reshape(128, 2 * N).astype(bf16)
        out = lax.dot_general(lhs, rhs, (((1,), (1,)), ((), ())), preferred_element_type=f32)
        out = out.reshape(NQ, 8, 128)
        for a in range(NA):
            accq = jnp.zeros((8, 128), f32)
            for p in range(8):
                q = 8 * a + p
                if q >= NQ:
                    break
                s = jnp.where(diag, out[q], 0.0)
                s = s + pltpu.roll(s, 1, 1); s = s + pltpu.roll(s, 2, 1); s = s + pltpu.roll(s, 4, 1)
                s = pltpu.roll(s, 121 + p, 1)
                accq = jnp.where((lane % 8) == p, s, accq)
            Kd[pl.ds(c0 + g * 8, 8), a * 128:(a + 1) * 128] = accq

    @pl.when(i == NSTEP - 1)
    def _():
        kdt = Kd[...].T
        for t in range(4):
            KdT[t] = kdt[:, t * 128:(t + 1) * 128]
        for t in range(4):
            UK[4 + t, 0:256, :] = KdT[t, 0:256, :]
            for mm in range(32, L // 8):
                rows = [KdT[t, SRC[8 * mm + s]:SRC[8 * mm + s] + 1, :] for s in range(8)]
                UK[4 + t, 8 * mm:8 * mm + 8, :] = jnp.concatenate(rows, axis=0)

        f1 = f1_ref[...]

        def s1(g, carry):
            b = pl.multiple_of(g * S, S)
            rhs = jnp.concatenate([
                jnp.concatenate([UK[t, pl.ds(64 * n1 + b, S), :] for n1 in range(32)], axis=0)
                for t in range(8)], axis=1).astype(bf16)
            out = jnp.dot(f1, rhs, preferred_element_type=f32)
            for t in range(8):
                for r in range(66):
                    Y1[t, pl.ds(64 * r + b, S), :] = out[S * r:S * r + S, t * 128:(t + 1) * 128]
            return carry
        lax.fori_loop(0, 64 // S, s1, 0, unroll=4)

        def s2(k1, carry):
            rr = pl.multiple_of(k1 * 128, 128)
            rhs = jnp.concatenate([Y1[t, pl.ds(rr, 128), :] for t in range(8)], axis=1).astype(bf16)
            X = jnp.dot(g_ref[k1], rhs, preferred_element_type=f32)
            Ur, Ui, Kr, Ki = X[:64, :512], X[64:, :512], X[:64, 512:], X[64:, 512:]
            Z = jnp.concatenate([Ur * Kr - Ui * Ki, Ur * Ki + Ui * Kr], axis=0).astype(bf16)
            qq = jnp.dot(gi_ref[k1], Z, preferred_element_type=f32)
            for t in range(4):
                Q[t, pl.ds(rr, 128), :] = qq[:, t * 128:(t + 1) * 128]
            return carry
        lax.fori_loop(0, 33, s2, 0, unroll=11)

        fi = fi_ref[...]

        def s3(g, carry):
            b = pl.multiple_of(g * S, S)
            rhs = jnp.concatenate([
                jnp.concatenate([Q[t, pl.ds(64 * r + b, S), :] for r in range(66)]
                                + [jnp.zeros((384 - 66 * S, 128), f32)], axis=0)
                for t in range(4)], axis=1).astype(bf16)
            yy = jnp.dot(fi, rhs, preferred_element_type=f32)
            for t in range(4):
                for n1 in range(32):
                    ACC[t, pl.ds(64 * n1 + b, S), :] += yy[S * n1:S * n1 + S, t * 128:(t + 1) * 128]
            return carry
        lax.fori_loop(0, 64 // S, s3, 0, unroll=4)

        o_ref[...] = jnp.concatenate([ACC[t] for t in range(4)], axis=1).astype(o_ref.dtype)


def _make_call():
    F1S, G, Gi, FiS = (jnp.asarray(a, dtype=bf16) for a in _dft_consts())
    full = lambda shape: pl.BlockSpec(shape, lambda i: (0,) * len(shape))

    def fn(A_u, A_A_re, A_A_im, A_B_re, A_B_im, A_C_re, A_C_im, A_log_dt, A_Dskip, B_x, B_w1, B_b1, B_w2, B_b2):
        x = A_u.reshape(L, D)
        out = pl.pallas_call(
            _kernel,
            grid=(NSTEP,),
            in_specs=[pl.BlockSpec((BLK, D), lambda i: (i, 0)),
                      full((D, 1)), full((D, N)), full((D, N)), full((D, N)), full((D, N)), full((D, N)), full((D, N)),
                      full((1, D)), full((D, F)), full((1, F)), full((F, D)), full((1, D)),
                      full((66 * S, 32 * S)), full((33, 128, 128)), full((33, 128, 128)), full((32 * S, 384))],
            out_specs=full((L, D)),
            out_shape=jax.ShapeDtypeStruct((L, D), bf16),
            scratch_shapes=[
                pltpu.VMEM((8, L, 128), f32),
                pltpu.VMEM((4, L, 128), f32),
                pltpu.VMEM((NQ, CH, 2 * N), f32),
                pltpu.VMEM((16, CH, 2 * N), f32),
                pltpu.VMEM((D, NA * 128), f32),
                pltpu.VMEM((4, NA * 128, 128), f32),
                pltpu.VMEM((8, 4224, 128), f32),
                pltpu.VMEM((4, 4224, 128), f32),
            ],
            compiler_params=pltpu.CompilerParams(dimension_semantics=("arbitrary",),
                                                 vmem_limit_bytes=110 * 1024 * 1024),
        )(x, A_log_dt.reshape(D, 1), A_A_re, A_A_im, A_B_re, A_B_im, A_C_re, A_C_im, A_Dskip.reshape(1, D),
          B_w1, B_b1.reshape(1, F), B_w2, B_b2.reshape(1, D), F1S, G, Gi, FiS)
        return out.reshape(1, L, D)
    return fn


_CALL = _make_call()


@jax.jit
def pallas_parallel_sum__ssm_conv_s4__mixer_channel_mlp__prompt_kernel(
    A_u, A_A_re, A_A_im, A_B_re, A_B_im, A_C_re, A_C_im, A_log_dt, A_Dskip, B_x, B_w1, B_b1, B_w2, B_b2
):
    return _CALL(A_u, A_A_re, A_A_im, A_B_re, A_B_im, A_C_re, A_C_im, A_log_dt, A_Dskip, B_x, B_w1, B_b1, B_w2, B_b2)
```

```python
import numpy as np
import jax
import jax.numpy as jnp
from jax import lax
import jax.experimental.pallas as pl
import jax.experimental.pallas.tpu as pltpu

L, D, N, F = 2048, 512, 128, 1792
BLK = 512
NSTEP = L // BLK
CH = D // NSTEP
S = 4
U2A, U2B = 11, 11
f32, bf16 = jnp.float32, jnp.bfloat16

ROWS = [(r, i) for i in (0, 1) for r in range(8)] + [(r, i) for i in (2, 3) for r in (0, 2, 4, 6)] + \
       [(r, i) for i in range(4, 8) for r in (0, 4)] + [(0, i) for i in range(8, 17)]
NQ = len(ROWS)
NA = (NQ + 7) // 8


def _bf16_round_int(v):
    if v < 256:
        return v
    sh = v.bit_length() - 8
    q, rem = v >> sh, v & ((1 << sh) - 1)
    half = 1 << (sh - 1)
    if rem > half or (rem == half and (q & 1)):
        q += 1
    return q << sh


def _src_rows():
    pos = {}
    for q, (r, i) in enumerate(ROWS):
        a, p = divmod(q, 8)
        for j in range(16):
            pos[8 * (16 * i + j) + r] = a * 128 + 8 * j + p
    return [pos[_bf16_round_int(l)] for l in range(L)]


SRC = _src_rows()


def _dft_consts():
    n1 = np.arange(32); k1 = np.arange(33)
    F1 = np.zeros((66, 32))
    ang = 2 * np.pi * np.outer(k1, n1) / 64
    F1[0::2] = np.cos(ang); F1[1::2] = -np.sin(ang)
    n2 = np.arange(64); k2 = np.arange(64)
    G = np.zeros((33, 128, 128)); Gi = np.zeros((33, 128, 128))
    for a in range(33):
        th = 2 * np.pi * np.outer(a + 64 * k2, n2) / 4096
        G[a, :64, :64] = np.cos(th); G[a, :64, 64:] = np.sin(th)
        G[a, 64:, :64] = -np.sin(th); G[a, 64:, 64:] = np.cos(th)
        thi = th.T
        Gi[a, :64, :64] = np.cos(thi); Gi[a, :64, 64:] = -np.sin(thi)
        Gi[a, 64:, :64] = np.sin(thi); Gi[a, 64:, 64:] = np.cos(thi)
    Fi = np.zeros((32, 66))
    for a in range(33):
        w = 1.0 if a in (0, 32) else 2.0
        ph = 2 * np.pi * a * n1 / 64
        Fi[:, 2 * a] = w * np.cos(ph) / 4096; Fi[:, 2 * a + 1] = -w * np.sin(ph) / 4096
    F1S = np.zeros((66 * S, 32 * S)); FiS = np.zeros((32 * S, 384))
    for a in range(S):
        F1S[a::S, a::S] = F1
        FiS[a::S, a:66 * S:S] = Fi
    return F1S, G, Gi, FiS


def _ln(a):
    m = jnp.mean(a, axis=-1, keepdims=True)
    c = a - m
    v = jnp.mean(c * c, axis=-1, keepdims=True)
    return c * lax.rsqrt(v + 1e-5)


def _cm(a, b):
    return (a[0] * b[0] - a[1] * b[1], a[0] * b[1] + a[1] * b[0])


def _kernel(x_ref, ldt_ref, are_ref, aim_ref, bre_ref, bim_ref, cre_ref, cim_ref, dk_ref,
            w1_ref, b1_ref, w2_ref, b2_ref, f1_ref, g_hbm, gi_hbm, fi_ref,
            o_ref,
            UK, ACC, E_s, F_s, Kd, KdT, Y1, Q, g_ref, gi_ref, sems, Zb, DT):
    i = pl.program_id(0)
    g_copy = pltpu.make_async_copy(g_hbm, g_ref, sems.at[0])
    gi_copy = pltpu.make_async_copy(gi_hbm, gi_ref, sems.at[1])

    @pl.when(i == 0)
    def _():
        g_copy.start()
        gi_copy.start()

    r0 = pl.multiple_of(i * BLK, BLK)
    c0 = pl.multiple_of(i * CH, CH)

    def kgen_pieces():
        dtr = jnp.exp(ldt_ref[...].reshape(1, D).astype(f32)).astype(bf16).astype(f32)
        DT[...] = jnp.broadcast_to(dtr, (N, D)).T
        dt = DT[pl.ds(c0, CH), :]
        ar = dt * are_ref[pl.ds(c0, CH), :].astype(f32)
        ai = dt * aim_ref[pl.ds(c0, CH), :].astype(f32)
        br = dt * bre_ref[pl.ds(c0, CH), :].astype(f32)
        bi = dt * bim_ref[pl.ds(c0, CH), :].astype(f32)
        c = _cm((cre_ref[pl.ds(c0, CH), :].astype(f32), cim_ref[pl.ds(c0, CH), :].astype(f32)), (br, bi))
        e = jnp.exp(ar)
        z = (e * jnp.cos(ai), e * jnp.sin(ai))
        z2 = _cm(z, z); z4 = _cm(z2, z2); w = _cm(z4, z4)
        one = jnp.ones_like(ar); zero = jnp.zeros_like(ar)
        Fj = (one, zero); F8 = None
        for j in range(16):
            F_s[j, :, 0:N] = Fj[0]; F_s[j, :, N:2 * N] = Fj[1]
            if j == 8:
                F8 = Fj
            if j < 15:
                Fj = _cm(Fj, w)
        yield
        w16 = _cm(F8, F8)
        cz = [c]
        for r in range(7):
            cz.append(_cm(cz[-1], z))
        Wi = (one, zero); q = 0
        for ii in range(17):
            for (r, i2) in ROWS:
                if i2 == ii:
                    E = _cm(cz[r], Wi)
                    E_s[q, :, 0:N] = E[0]; E_s[q, :, N:2 * N] = -E[1]
                    q += 1
            if ii < 16:
                Wi = _cm(Wi, w16)
            if ii in (1, 7):
                yield
        yield
        lane = lax.broadcasted_iota(jnp.int32, (8, 128), 1)
        sub = lax.broadcasted_iota(jnp.int32, (8, 128), 0)
        diag = (lane % 8) == sub
        for g in range(CH // 8):
            lhs = E_s[:, g * 8:(g + 1) * 8, :].reshape(NQ * 8, 2 * N).astype(bf16)
            rhs = F_s[:, g * 8:(g + 1) * 8, :].reshape(128, 2 * N).astype(bf16)
            out = lax.dot_general(lhs, rhs, (((1,), (1,)), ((), ())), preferred_element_type=f32)
            out = out.reshape(NQ, 8, 128)
            for a in range(NA):
                tt = None
                for p in range(8):
                    q = 8 * a + p
                    if q >= NQ:
                        break
                    s = jnp.where(diag, out[q], 0.0)
                    if p:
                        s = pltpu.roll(s, p, 1)
                    tt = s if tt is None else tt + s
                for bit in (1, 2, 4):
                    tt = jnp.where((sub & bit) != 0, pltpu.roll(tt, 128 - bit, 1), tt)
                Kd[pl.ds(c0 + g * 8, 8), a * 128:(a + 1) * 128] = tt
            if g % 2 == 1:
                yield

    gen = kgen_pieces()
    x = x_ref[...].astype(f32)
    xn = _ln(x).astype(bf16).astype(f32)
    y = _ln(xn).astype(bf16)
    acc = x + xn * dk_ref[...].reshape(1, D).astype(f32) + b2_ref[...].reshape(1, D).astype(f32)
    FC = 256
    for cc in range(F // FC):
        h = jnp.dot(y, w1_ref[:, cc * FC:(cc + 1) * FC], preferred_element_type=f32) + b1_ref[cc * FC:(cc + 1) * FC].reshape(1, FC).astype(f32)
        next(gen, None)
        h = jax.nn.gelu(h, approximate=True).astype(bf16)
        acc = acc + jnp.dot(h, w2_ref[cc * FC:(cc + 1) * FC, :], preferred_element_type=f32)
        next(gen, None)
    for _ in gen:
        pass
    for t in range(4):
        UK[t, pl.ds(r0, BLK), :] = xn[:, t * 128:(t + 1) * 128]
        ACC[t, pl.ds(r0, BLK), :] = acc[:, t * 128:(t + 1) * 128]

    @pl.when(i == NSTEP - 1)
    def _():
        g_copy.wait()
        gi_copy.wait()
        kdt = Kd[...].T
        for t in range(4):
            KdT[t] = kdt[:, t * 128:(t + 1) * 128]
        for t in range(4):
            UK[4 + t, 0:256, :] = KdT[t, 0:256, :]
            for mm in range(32, L // 8):
                rows = [KdT[t, SRC[8 * mm + s]:SRC[8 * mm + s] + 1, :] for s in range(8)]
                UK[4 + t, 8 * mm:8 * mm + 8, :] = jnp.concatenate(rows, axis=0)

        f1 = f1_ref[...]

        def s1(g, carry):
            b = pl.multiple_of(g * S, S)
            rhs = jnp.concatenate([
                jnp.concatenate([UK[t, pl.ds(64 * n1 + b, S), :] for n1 in range(32)], axis=0)
                for t in range(8)], axis=1).astype(bf16)
            out = jnp.dot(f1, rhs, preferred_element_type=f32)
            for t in range(8):
                for r in range(66):
                    Y1[t, pl.ds(64 * r + b, S), :] = out[S * r:S * r + S, t * 128:(t + 1) * 128]
            return carry
        lax.fori_loop(0, 64 // S, s1, 0, unroll=8)

        def s2a(k1, carry):
            rr = pl.multiple_of(k1 * 128, 128)
            rhs = jnp.concatenate([Y1[t, pl.ds(rr, 128), :] for t in range(8)], axis=1).astype(bf16)
            X = jnp.dot(g_ref[k1], rhs, preferred_element_type=f32)
            Ur, Ui, Kr, Ki = X[:64, :512], X[64:, :512], X[:64, 512:], X[64:, 512:]
            Zb[pl.ds(rr, 128), :] = jnp.concatenate([Ur * Kr - Ui * Ki, Ur * Ki + Ui * Kr], axis=0).astype(bf16)
            return carry
        lax.fori_loop(0, 33, s2a, 0, unroll=U2A)

        def s2b(k1, carry):
            rr = pl.multiple_of(k1 * 128, 128)
            qq = jnp.dot(gi_ref[k1], Zb[pl.ds(rr, 128), :], preferred_element_type=f32)
            for t in range(4):
                Q[t, pl.ds(rr, 128), :] = qq[:, t * 128:(t + 1) * 128]
            return carry
        lax.fori_loop(0, 33, s2b, 0, unroll=U2B)

        fi = fi_ref[...]

        def s3(g, carry):
            b = pl.multiple_of(g * S, S)
            rhs = jnp.concatenate([
                jnp.concatenate([Q[t, pl.ds(64 * r + b, S), :] for r in range(66)]
                                + [jnp.zeros((384 - 66 * S, 128), f32)], axis=0)
                for t in range(4)], axis=1).astype(bf16)
            yy = jnp.dot(fi, rhs, preferred_element_type=f32)
            for t in range(4):
                for n1 in range(32):
                    ACC[t, pl.ds(64 * n1 + b, S), :] += yy[S * n1:S * n1 + S, t * 128:(t + 1) * 128]
            return carry
        lax.fori_loop(0, 64 // S, s3, 0, unroll=8)

        o_ref[...] = jnp.concatenate([ACC[t] for t in range(4)], axis=1).astype(o_ref.dtype)


def _make_call():
    F1S, G, Gi, FiS = (jnp.asarray(a, dtype=bf16) for a in _dft_consts())
    full = lambda shape: pl.BlockSpec(shape, lambda i: (0,) * len(shape))
    anyspec = pl.BlockSpec(memory_space=pl.ANY)

    def fn(A_u, A_A_re, A_A_im, A_B_re, A_B_im, A_C_re, A_C_im, A_log_dt, A_Dskip, B_x, B_w1, B_b1, B_w2, B_b2):
        x = A_u.reshape(L, D)
        out = pl.pallas_call(
            _kernel,
            grid=(NSTEP,),
            in_specs=[pl.BlockSpec((BLK, D), lambda i: (i, 0)),
                      full((D,)), full((D, N)), full((D, N)), full((D, N)), full((D, N)), full((D, N)), full((D, N)),
                      full((D,)), full((D, F)), full((F,)), full((F, D)), full((D,)),
                      full((66 * S, 32 * S)), anyspec, anyspec, full((32 * S, 384))],
            out_specs=full((L, D)),
            out_shape=jax.ShapeDtypeStruct((L, D), bf16),
            scratch_shapes=[
                pltpu.VMEM((8, L, 128), f32),
                pltpu.VMEM((4, L, 128), f32),
                pltpu.VMEM((NQ, CH, 2 * N), f32),
                pltpu.VMEM((16, CH, 2 * N), f32),
                pltpu.VMEM((D, NA * 128), f32),
                pltpu.VMEM((4, NA * 128, 128), f32),
                pltpu.VMEM((8, 4224, 128), f32),
                pltpu.VMEM((4, 4224, 128), f32),
                pltpu.VMEM((33, 128, 128), bf16), pltpu.VMEM((33, 128, 128), bf16),
                pltpu.SemaphoreType.DMA((2,)),
                pltpu.VMEM((4224, 512), bf16),
                pltpu.VMEM((D, N), f32),
            ],
            compiler_params=pltpu.CompilerParams(dimension_semantics=("arbitrary",),
                                                 vmem_limit_bytes=110 * 1024 * 1024),
        )(x, A_log_dt, A_A_re, A_A_im, A_B_re, A_B_im, A_C_re, A_C_im, A_Dskip,
          B_w1, B_b1, B_w2, B_b2, F1S, G, Gi, FiS)
        return out.reshape(1, L, D)
    return fn


_CALL = _make_call()


@jax.jit
def pallas_parallel_sum__ssm_conv_s4__mixer_channel_mlp__prompt_kernel(
    A_u, A_A_re, A_A_im, A_B_re, A_B_im, A_C_re, A_C_im, A_log_dt, A_Dskip, B_x, B_w1, B_b1, B_w2, B_b2
):
    return _CALL(A_u, A_A_re, A_A_im, A_B_re, A_B_im, A_C_re, A_C_im, A_log_dt, A_Dskip, B_x, B_w1, B_b1, B_w2, B_b2)
```
